```python
import os as _os
_os.environ.setdefault("JAX_PLATFORMS", "cpu")
import jax
import jax.numpy as jnp

def _softmax(x, axis=-1):
    return jax.nn.softmax(x, axis=axis)
def _gelu(x):
    return jax.nn.gelu(x, approximate=True)
def _silu(x):
    return jax.nn.silu(x)
def _sigmoid(x):
    return jax.nn.sigmoid(x)
def _layernorm(x, axis=-1, eps=1e-5):
    m = jnp.mean(x, axis=axis, keepdims=True)
    v = jnp.var(x, axis=axis, keepdims=True)
    return (x - m) / jnp.sqrt(v + eps)
def _scatter_add(tgt, idx, src, axis=0):
    return tgt.at[idx].add(src)
def _segment_sum(src, seg, n):
    return jax.ops.segment_sum(src, seg, n)
class _Rng:
    def __init__(self, key):
        self._k = key
    def _next(self):
        self._k, sub = jax.random.split(self._k)
        return sub
    def normal(self, shape):
        return jax.random.normal(self._next(), shape, dtype=jnp.bfloat16)
    def randint(self, lo, hi, shape):
        return jax.random.randint(self._next(), shape, lo, hi, dtype=jnp.int32)
    def uniform(self, shape, lo=0.0, hi=1.0):
        return jax.random.uniform(self._next(), shape, jnp.bfloat16, lo, hi)
    def permutation(self, n):
        return jax.random.permutation(self._next(), n)


kernel_name = 'standalone__gqa_block_cached__near_ridge'

def setup_inputs():
    _rng = _Rng(jax.random.key(int.from_bytes(__import__("os").urandom(4), "little")))
    _w = (lambda a: (lambda t: t.astype(jnp.bfloat16) if jnp.issubdtype(t.dtype, jnp.floating) else t)(jnp.asarray(a)))
    B, Sq, D = 16, 128, 576
    Hq, Hkv, Sk, Dh = 32, 16, 1024, 128
    assert Hq % Hkv == 0, (Hq, Hkv)
    return {
        "x": _w((lambda *s: _rng.normal(s) * 0.8)(B, Sq, D)),
        "k_cache": _w((lambda *s: _rng.normal(s) * 0.8)(B, Hkv, Sk, Dh)),
        "v_cache": _w((lambda *s: _rng.normal(s) * 0.05)(B, Hkv, Sk, Dh)),
        "wq": _w((lambda *s: _rng.normal(s) * 0.8)(D, Hq * Dh) * (D ** -0.5)),
        "wo": _w((lambda *s: _rng.normal(s) * 0.05)(Hq * Dh, D) * ((Hq * Dh) ** -0.5)),
    }

def reference(x, k_cache, v_cache, wq, wo):
    B, Sq, D = x.shape
    Hq, Dh = 32, 128
    Hkv = k_cache.shape[1]
    rep = Hq // Hkv
    q = (lambda x, *d: x.transpose(*d))((x @ wq).reshape(B, Sq, Hq, Dh), 0, 2, 1, 3)
    k = jnp.repeat(k_cache, rep, axis=1)
    v = jnp.repeat(v_cache, rep, axis=1)
    scores = jnp.einsum("bhqd,bhkd->bhqk", q, k) * (Dh ** -0.5)
    p = _softmax(scores, axis=-1)
    o = jnp.einsum("bhqk,bhkd->bhqd", p, v)
    return (lambda x, *d: x.transpose(*d))(o, 0, 2, 1, 3).reshape(B, Sq, Hq * Dh) @ wo
```

```python
import jax
import jax.numpy as jnp
import jax.experimental.pallas as pl
import jax.experimental.pallas.tpu as pltpu

_BB = 4


def _kernel(x_ref, k_ref, v_ref, wq_ref, wo_ref, o_ref, acc_ref):
    bb = _BB
    h = pl.program_id(0)
    bi = pl.program_id(1)
    nh = pl.num_programs(0)
    Sq, D = x_ref.shape[1], x_ref.shape[2]
    Dh = k_ref.shape[-1]
    scale = Dh ** -0.5
    xb = x_ref[pl.ds(bi * bb, bb)].reshape(bb * Sq, D)
    q = jnp.dot(xb, wq_ref[...], preferred_element_type=jnp.float32)
    q = (q * scale).astype(jnp.bfloat16)
    outs = []
    for j in range(bb):
        qj = q[j * Sq:(j + 1) * Sq]
        q2 = jnp.concatenate([qj[:, :Dh], qj[:, Dh:]], axis=0)
        s = jax.lax.dot_general(q2, k_ref[j, 0], (((1,), (1,)), ((), ())),
                                preferred_element_type=jnp.float32)
        m = jnp.max(s, axis=-1, keepdims=True)
        p = jnp.exp(s - m)
        l = jnp.sum(p, axis=-1, keepdims=True)
        o = jnp.dot(p.astype(jnp.bfloat16), v_ref[j, 0], preferred_element_type=jnp.float32)
        o = (o / l).astype(jnp.bfloat16)
        outs.append(jnp.concatenate([o[:Sq], o[Sq:]], axis=1))
    oa = jnp.concatenate(outs, axis=0)
    y = jnp.dot(oa, wo_ref[...], preferred_element_type=jnp.float32)
    rows = pl.ds(bi * bb * Sq, bb * Sq)

    @pl.when(h == 0)
    def _():
        acc_ref[rows, :] = y

    @pl.when(h > 0)
    def _():
        acc_ref[rows, :] += y

    @pl.when(h == nh - 1)
    def _():
        o_ref[pl.ds(bi * bb, bb)] = acc_ref[rows, :].reshape(bb, Sq, D).astype(o_ref.dtype)


@jax.jit
def pallas_standalone__gqa_block_cached__near_ridge_kernel(
    x: jax.Array,
    k_cache: jax.Array,
    v_cache: jax.Array,
    wq: jax.Array,
    wo: jax.Array,
):
    bb = _BB
    B, Sq, D = x.shape
    _, Hkv, Sk, Dh = k_cache.shape
    rep = wq.shape[1] // Dh // Hkv
    return pl.pallas_call(
        _kernel,
        grid=(Hkv, B // bb),
        in_specs=[
            pl.BlockSpec((B, Sq, D), lambda h, b: (0, 0, 0)),
            pl.BlockSpec((bb, 1, Sk, Dh), lambda h, b: (b, h, 0, 0)),
            pl.BlockSpec((bb, 1, Sk, Dh), lambda h, b: (b, h, 0, 0)),
            pl.BlockSpec((D, rep * Dh), lambda h, b: (0, h)),
            pl.BlockSpec((rep * Dh, D), lambda h, b: (h, 0)),
        ],
        out_specs=pl.BlockSpec((B, Sq, D), lambda h, b: (0, 0, 0)),
        out_shape=jax.ShapeDtypeStruct((B, Sq, D), x.dtype),
        scratch_shapes=[pltpu.VMEM((B * Sq, D), jnp.float32)],
        compiler_params=pltpu.CompilerParams(
            dimension_semantics=("arbitrary", "arbitrary"),
            vmem_limit_bytes=100 * 1024 * 1024),
    )(x, k_cache, v_cache, wq, wo)
```

```python
import jax
import jax.numpy as jnp
import jax.experimental.pallas as pl
import jax.experimental.pallas.tpu as pltpu

_BB = 8
_RC = 32


def _kernel(xt_ref, k0_ref, kn_ref, v_ref, wq0_ref, wqn_ref, wot_ref, o_ref,
            xs_ref, acc_ref, p_scr, l_scr):
    bb, rc = _BB, _RC
    h = pl.program_id(0)
    bi = pl.program_id(1)
    nh = pl.num_programs(0)
    nb = pl.num_programs(1)
    t = h * nb + bi
    B, D, Sq = xt_ref.shape
    Dh = k0_ref.shape[-1]
    R = bb * Sq
    scale = Dh ** -0.5

    def qproj(rows, w_ref):
        q = jnp.dot(xs_ref[rows, :], w_ref[...], preferred_element_type=jnp.float32)
        return (q * scale).astype(jnp.bfloat16)

    def qk(q, j, kref):
        qj = q[j * Sq:(j + 1) * Sq]
        q2 = jnp.concatenate([qj[:, :Dh], qj[:, Dh:]], axis=0)
        return jax.lax.dot_general(q2, kref[j, 0], (((1,), (1,)), ((), ())),
                                   preferred_element_type=jnp.float32)

    def softmax_store(s, j):
        for c in range(s.shape[0] // rc):
            sc = s[c * rc:(c + 1) * rc]
            m = jnp.max(sc, axis=-1, keepdims=True)
            p = jnp.exp(sc - m)
            l_scr[j, pl.ds(c * rc, rc), :] = jnp.sum(p, axis=-1, keepdims=True)
            p_scr[j, pl.ds(c * rc, rc), :] = p.astype(jnp.bfloat16)

    @pl.when(t == 0)
    def _():
        for j in range(B):
            xs_ref[pl.ds(j * Sq, Sq), :] = xt_ref[j].T
        q0 = qproj(pl.ds(0, R), wq0_ref)
        for j in range(bb):
            softmax_store(qk(q0, j, k0_ref), j)

    bn = jnp.where(bi == nb - 1, 0, bi + 1)
    rows_n = pl.ds(pl.multiple_of(bn * R, R), R)

    def pv(j):
        o = jnp.dot(p_scr[j], v_ref[j, 0], preferred_element_type=jnp.float32)
        o = (o / l_scr[j]).astype(jnp.bfloat16)
        return jnp.concatenate([o[:Sq].T, o[Sq:].T], axis=0)

    qn = qproj(rows_n, wqn_ref)
    outs = [pv(0)]
    s_prev = qk(qn, 0, kn_ref)
    for j in range(1, bb):
        outs.append(pv(j))
        softmax_store(s_prev, j - 1)
        s_prev = qk(qn, j, kn_ref)
    oat = jnp.concatenate(outs, axis=1)
    y = jnp.dot(wot_ref[...], oat, preferred_element_type=jnp.float32)
    acc_ref[bi] = jnp.where(h > 0, acc_ref[bi], 0.0) + y
    softmax_store(s_prev, bb - 1)

    @pl.when(t == nh * nb - 1)
    def _():
        for j in range(B):
            o_ref[j] = acc_ref[j // bb, :, pl.ds((j % bb) * Sq, Sq)].astype(o_ref.dtype)


@jax.jit
def pallas_standalone__gqa_block_cached__near_ridge_kernel(
    x: jax.Array,
    k_cache: jax.Array,
    v_cache: jax.Array,
    wq: jax.Array,
    wo: jax.Array,
):
    bb = _BB
    B, Sq, D = x.shape
    _, Hkv, Sk, Dh = k_cache.shape
    rep = wq.shape[1] // Dh // Hkv
    nb = B // bb
    xt = x.transpose(0, 2, 1)
    wot = wo.T

    def next_h(h, b):
        return jnp.minimum(jnp.where(b == nb - 1, h + 1, h), Hkv - 1)

    def next_b(h, b):
        return jnp.where(b == nb - 1, 0, b + 1)

    ot = pl.pallas_call(
        _kernel,
        grid=(Hkv, nb),
        in_specs=[
            pl.BlockSpec((B, D, Sq), lambda h, b: (0, 0, 0)),
            pl.BlockSpec((bb, 1, Sk, Dh), lambda h, b: (0, 0, 0, 0)),
            pl.BlockSpec((bb, 1, Sk, Dh), lambda h, b: (next_b(h, b), next_h(h, b), 0, 0)),
            pl.BlockSpec((bb, 1, Sk, Dh), lambda h, b: (b, h, 0, 0)),
            pl.BlockSpec((D, rep * Dh), lambda h, b: (0, 0)),
            pl.BlockSpec((D, rep * Dh), lambda h, b: (0, next_h(h, b))),
            pl.BlockSpec((D, rep * Dh), lambda h, b: (0, h)),
        ],
        out_specs=pl.BlockSpec((B, D, Sq), lambda h, b: (0, 0, 0)),
        out_shape=jax.ShapeDtypeStruct((B, D, Sq), x.dtype),
        scratch_shapes=[pltpu.VMEM((B * Sq, D), jnp.bfloat16),
                        pltpu.VMEM((nb, D, bb * Sq), jnp.float32),
                        pltpu.VMEM((bb, rep * Sq, Sk), jnp.bfloat16),
                        pltpu.VMEM((bb, rep * Sq, 1), jnp.float32)],
        compiler_params=pltpu.CompilerParams(
            dimension_semantics=("arbitrary", "arbitrary"),
            vmem_limit_bytes=100 * 1024 * 1024),
    )(xt, k_cache, k_cache, v_cache, wq, wq, wot)
    return ot.transpose(0, 2, 1)
```

```python
import jax
import jax.numpy as jnp
import jax.experimental.pallas as pl
import jax.experimental.pallas.tpu as pltpu

_BB = 8
_RC = 32


def _kernel(xt_ref, k_hbm, v_hbm, wq0_ref, wqn_ref, wot_ref, o_ref,
           xs_ref, acc_ref, p_scr, l_scr, kbuf, vbuf, ksem, vsem):
    bb, rc = _BB, _RC
    h = pl.program_id(0)
    bi = pl.program_id(1)
    nh = pl.num_programs(0)
    nb = pl.num_programs(1)
    t = h * nb + bi
    T = nh * nb
    B, D, Sq = xt_ref.shape
    Dh = 128
    R = bb * Sq
    scale = Dh ** -0.5

    def kv_copy(hbm, buf, sem, tt):
        hh = tt // nb
        b0 = (tt % nb) * bb
        slot = tt % 2
        return pltpu.make_async_copy(hbm.at[pl.ds(b0, bb), hh], buf.at[slot], sem.at[slot])

    def qproj(rows, w_ref):
        q = jnp.dot(xs_ref[rows, :], w_ref[...], preferred_element_type=jnp.float32)
        return (q * scale).astype(jnp.bfloat16)

    def qk(q, j, slot):
        qj = q[j * Sq:(j + 1) * Sq]
        q2 = jnp.concatenate([qj[:, :Dh], qj[:, Dh:]], axis=0)
        return jax.lax.dot_general(q2, kbuf[slot, j], (((1,), (1,)), ((), ())),
                                   preferred_element_type=jnp.float32)

    def softmax_store(s, j):
        for c in range(s.shape[0] // rc):
            sc = s[c * rc:(c + 1) * rc]
            m = jnp.max(sc, axis=-1, keepdims=True)
            p = jnp.exp(sc - m)
            l_scr[j, pl.ds(c * rc, rc), :] = jnp.sum(p, axis=-1, keepdims=True)
            p_scr[j, pl.ds(c * rc, rc), :] = p.astype(jnp.bfloat16)

    @pl.when(t == 0)
    def _():
        kv_copy(k_hbm, kbuf, ksem, 0).start()
        kv_copy(k_hbm, kbuf, ksem, 1).start()
        kv_copy(v_hbm, vbuf, vsem, 0).start()
        for j in range(B):
            xs_ref[pl.ds(j * Sq, Sq), :] = xt_ref[j].T
        q0 = qproj(pl.ds(0, R), wq0_ref)
        kv_copy(k_hbm, kbuf, ksem, 0).wait()
        for j in range(bb):
            softmax_store(qk(q0, j, 0), j)

    kv_copy(v_hbm, vbuf, vsem, t).wait()

    @pl.when(t + 1 < T)
    def _():
        kv_copy(k_hbm, kbuf, ksem, t + 1).wait()
        kv_copy(v_hbm, vbuf, vsem, t + 1).start()

    @pl.when(t + 2 < T)
    def _():
        kv_copy(k_hbm, kbuf, ksem, t + 2).start()

    vslot = t % 2
    kslot = (t + 1) % 2
    bn = jnp.where(bi == nb - 1, 0, bi + 1)
    rows_n = pl.ds(pl.multiple_of(bn * R, R), R)

    def pv(j):
        o = jnp.dot(p_scr[j], vbuf[vslot, j], preferred_element_type=jnp.float32)
        o = (o / l_scr[j]).astype(jnp.bfloat16)
        return jnp.concatenate([o[:Sq].T, o[Sq:].T], axis=0)

    def outproj(outs):
        oat = jnp.concatenate(outs, axis=1)
        y = jnp.dot(wot_ref[...], oat, preferred_element_type=jnp.float32)
        acc_ref[bi] = jnp.where(h > 0, acc_ref[bi], 0.0) + y

    @pl.when(t < T - 1)
    def _():
        qn = qproj(rows_n, wqn_ref)
        outs = [pv(0)]
        s_prev = qk(qn, 0, kslot)
        for j in range(1, bb):
            outs.append(pv(j))
            softmax_store(s_prev, j - 1)
            s_prev = qk(qn, j, kslot)
        outproj(outs)
        softmax_store(s_prev, bb - 1)

    @pl.when(t == T - 1)
    def _():
        outproj([pv(j) for j in range(bb)])

    @pl.when(t == T - 1)
    def _():
        for j in range(B):
            o_ref[j] = acc_ref[j // bb, :, pl.ds((j % bb) * Sq, Sq)].astype(o_ref.dtype)


@jax.jit
def pallas_standalone__gqa_block_cached__near_ridge_kernel(
    x: jax.Array,
    k_cache: jax.Array,
    v_cache: jax.Array,
    wq: jax.Array,
    wo: jax.Array,
):
    bb = _BB
    B, Sq, D = x.shape
    _, Hkv, Sk, Dh = k_cache.shape
    rep = wq.shape[1] // Dh // Hkv
    nb = B // bb
    xt = x.transpose(0, 2, 1)
    wot = wo.T

    def next_h(h, b):
        return jnp.minimum(jnp.where(b == nb - 1, h + 1, h), Hkv - 1)

    ot = pl.pallas_call(
        _kernel,
        grid=(Hkv, nb),
        in_specs=[
            pl.BlockSpec((B, D, Sq), lambda h, b: (0, 0, 0)),
            pl.BlockSpec(memory_space=pl.ANY),
            pl.BlockSpec(memory_space=pl.ANY),
            pl.BlockSpec((D, rep * Dh), lambda h, b: (0, 0)),
            pl.BlockSpec((D, rep * Dh), lambda h, b: (0, next_h(h, b))),
            pl.BlockSpec((D, rep * Dh), lambda h, b: (0, h)),
        ],
        out_specs=pl.BlockSpec((B, D, Sq), lambda h, b: (0, 0, 0)),
        out_shape=jax.ShapeDtypeStruct((B, D, Sq), x.dtype),
        scratch_shapes=[pltpu.VMEM((B * Sq, D), jnp.bfloat16),
                        pltpu.VMEM((nb, D, bb * Sq), jnp.float32),
                        pltpu.VMEM((bb, rep * Sq, Sk), jnp.bfloat16),
                        pltpu.VMEM((bb, rep * Sq, 1), jnp.float32),
                        pltpu.VMEM((2, bb, Sk, Dh), jnp.bfloat16),
                        pltpu.VMEM((2, bb, Sk, Dh), jnp.bfloat16),
                        pltpu.SemaphoreType.DMA((2,)),
                        pltpu.SemaphoreType.DMA((2,))],
        compiler_params=pltpu.CompilerParams(
            dimension_semantics=("arbitrary", "arbitrary"),
            vmem_limit_bytes=100 * 1024 * 1024),
    )(xt, k_cache, v_cache, wq, wq, wot)
    return ot.transpose(0, 2, 1)
```
